```python
import jax
import jax.numpy as jnp

def _softmax(x, axis=-1):
    return jax.nn.softmax(x, axis=axis)
def _gelu(x):
    return jax.nn.gelu(x, approximate=True)
def _silu(x):
    return jax.nn.silu(x)
def _sigmoid(x):
    return jax.nn.sigmoid(x)
def _layernorm(x, axis=-1, eps=1e-5):
    m = jnp.mean(x, axis=axis, keepdims=True)
    v = jnp.var(x, axis=axis, keepdims=True)
    return (x - m) / jnp.sqrt(v + eps)
def _scatter_add(tgt, idx, src, axis=0):
    return tgt.at[idx].add(src)
def _segment_sum(src, seg, n):
    return jax.ops.segment_sum(src, seg, n)
class _Rng:
    def __init__(self, key):
        self._k = key
    def _next(self):
        self._k, sub = jax.random.split(self._k)
        return sub
    def normal(self, shape):
        return jax.random.normal(self._next(), shape, dtype=jnp.bfloat16)
    def randint(self, lo, hi, shape):
        return jax.random.randint(self._next(), shape, lo, hi, dtype=jnp.int32)
    def uniform(self, shape, lo=0.0, hi=1.0):
        return jax.random.uniform(self._next(), shape, jnp.bfloat16, lo, hi)
    def permutation(self, n):
        return jax.random.permutation(self._next(), n)


kernel_name = 'standalone__gqa_block_cached__near_ridge'

def _fwd_setup_inputs():
    _rng = _Rng(jax.random.key(int.from_bytes(__import__("os").urandom(4), "little")))
    _w = (lambda a: (lambda t: t.astype(jnp.bfloat16) if jnp.issubdtype(t.dtype, jnp.floating) else t)(jnp.asarray(a)))
    B, Sq, D = 16, 64, 640
    Hq, Hkv, Sk, Dh = 32, 32, 512, 192
    assert Hq % Hkv == 0, (Hq, Hkv)
    return {
        "x": _w((lambda *s: _rng.normal(s) * 0.05)(B, Sq, D)),
        "k_cache": _w((lambda *s: _rng.normal(s) * 0.05)(B, Hkv, Sk, Dh)),
        "v_cache": _w((lambda *s: _rng.normal(s) * 0.05)(B, Hkv, Sk, Dh)),
        "wq": _w((lambda *s: _rng.normal(s) * 0.05)(D, Hq * Dh) * (D ** -0.5)),
        "wo": _w((lambda *s: _rng.normal(s) * 0.05)(Hq * Dh, D) * ((Hq * Dh) ** -0.5)),
    }

def _fwd_reference(x, k_cache, v_cache, wq, wo):
    B, Sq, D = x.shape
    Hq, Dh = 32, 192
    Hkv = k_cache.shape[1]
    rep = Hq // Hkv
    q = (lambda x, *d: x.transpose(*d))((x @ wq).reshape(B, Sq, Hq, Dh), 0, 2, 1, 3)
    k = jnp.repeat(k_cache, rep, axis=1)
    v = jnp.repeat(v_cache, rep, axis=1)
    scores = jnp.einsum("bhqd,bhkd->bhqk", q, k) * (Dh ** -0.5)
    p = _softmax(scores, axis=-1)
    o = jnp.einsum("bhqk,bhkd->bhqd", p, v)
    return (lambda x, *d: x.transpose(*d))(o, 0, 2, 1, 3).reshape(B, Sq, Hq * Dh) @ wo


def setup_inputs():
    _inp = _fwd_setup_inputs()
    _gk = jax.random.fold_in(jax.random.key(int.from_bytes(__import__("os").urandom(4), "little")), 2**31 - 1)
    _shapes = [[16, 64, 640]]
    _dtypes = ['bfloat16']
    _gks = jax.random.split(_gk, len(_shapes))
    _gs = [jax.random.normal(k, s, dtype=jnp.dtype(d)) * 0.05 for k, s, d in zip(_gks, _shapes, _dtypes)]
    _inp["grad_out"] = _gs[0]
    return _inp

def reference(x, k_cache, v_cache, wq, wo, grad_out):
    _const = dict()
    def _f(*_d):
        return _fwd_reference(**{'x': _d[0], 'k_cache': _d[1], 'v_cache': _d[2], 'wq': _d[3], 'wo': _d[4], **_const})
    _out, _vjp = jax.vjp(_f, x, k_cache, v_cache, wq, wo)
    _grads = _vjp(grad_out)
    _out0 = jnp.asarray(_out)
    return (_out0, *[jnp.asarray(_g) for _g in _grads])
```

```python
import contextlib
import math

import jax
import jax.numpy as jnp
from jax import lax
import jax.experimental.pallas as pl
import jax.experimental.pallas.tpu as pltpu

B, SQ, D = 16, 64, 640
H, SK, DH = 32, 512, 192
NP = H // 2
PW = 2 * DH
NSTEP = 4 * NP
NBLK = NSTEP // 2
HEAD = 4
DB = 3
NS = 4
OFF = 255

NN = (((1,), (0,)), ((), ()))
NT = (((1,), (1,)), ((), ()))
TN = (((0,), (0,)), ((), ()))
F32, BF16 = jnp.float32, jnp.bfloat16


def _dot(a, b, dims=NN):
    return lax.dot_general(a, b, dims, preferred_element_type=F32)


def _runs(size, stop, start=0):
    return [(a, min(size, stop - a)) for a in range(start, stop, size)]


def _make_plan(phases, dw_steps, defer):
    reading = [n % 2 == 0 for n, length in enumerate(phases) for _ in range(length)]
    assert len(reading) == NSTEP
    switches = [t for t in range(NSTEP - 1) if reading[t] != reading[t + 1]]

    started = [(1, 0, 2, 0)]
    for t in range(NSTEP):
        r, w, m, d = started[-1]
        if reading[t]:
            r, m = r + 1, min(m + 1, 2 * NP)
        elif 2 * w + 2 <= t:
            w += 1
        if t in dw_steps:
            d += 1
            assert not reading[t] and DB * d <= t // 4
        started.append((r, w, m, d))
    assert started[-1] == (NBLK, NBLK - 1, 2 * NP, (NP - 1) // DB) and (NP - 1) % DB == 0

    stops = [t for t in range(NSTEP) if t < HEAD or t % 2]
    done = [(1, 0, 2, 0)]
    for t in range(NSTEP):
        r, w, m, d = done[-1]
        if t in stops[:-1]:
            until = stops[stops.index(t) + 1]
            r = max(r, until // 2 + 1, started[t + 1][0] - 2)
            m = max(m, min(2 * ((until + 1) // 4 + 1), 2 * NP), started[t + 1][2] - 2)
            w = max(w, 2 * started[t][1])
            if reading[t + 1] and not reading[t]:
                w = max(w, 2 * started[t + 1][1] - 1)
            d = max(d, started[max(t - 1, 0)][3])
        done.append((r, w, m, d))
        sr, sw, sm, sd = started[t + 1]
        assert r <= sr and w <= 2 * sw and m <= sm and d <= sd
        assert max(sr - done[t][0], sw + (t >= NSTEP - 2) - done[t][1] // 2, sm - done[t][2]) <= NS
    for n in range(len(defer)):
        assert done[switches[2 * n + 1] + 1][0] < started[switches[2 * n] + 1][0]

    n_kv = max(started[t + 1][0] - t // 2 for t in range(NSTEP))
    n_dkv = max(t // 2 + 1 - done[t][1] // 2 for t in range(NSTEP))
    n_w = max((started[t + 1][2] + 1) // 2 - t // 4 for t in range(NSTEP))
    n_dw = DB * max(t // 4 // DB + 1 - done[t][3] for t in range(NSTEP))

    table = []
    for t in range(NSTEP):
        (r, w, m, d), (r1, w1, m1, d1) = started[t], started[t + 1]
        skip = sum(k for n, k in enumerate(defer) if t == switches[2 * n])
        late = sum(k for n, k in enumerate(defer) if t == switches[2 * n + 1] + 1)
        table.append(dict(
            r_blk=r, r_slot=r % n_kv, r_skip=skip if r1 > r else OFF, w_blk=w if w1 > w else OFF,
            w_slot=w % n_dkv, l_num=late, l_slot=(r - 1) % n_kv, kv_slot=t // 2 % n_kv,
            dkv_slot=t // 2 % n_dkv, dw_slot=t // 4 % n_dw, w_next=min(t + 1, NSTEP - 1) // 4 % n_w,
            m_mat=m if m1 > m else OFF, m_slot=m // 2 % n_w, d_num=d if d1 > d else OFF, d_slot=DB * d % n_dw))
    return table, done, (n_kv, n_dkv, n_w, n_dw)


def _pack(fields):
    word = sum(v << (8 * n) for n, v in enumerate(fields))
    return word - (1 << 32) if word >= 1 << 31 else word


def make(phases=(12, 10, 10, 10, 9, 13), dw_steps=(12, 32, 51, 60, 61), defer=(5, 3),
         drip=(2, 24), bulk_rows=96, out_rows=40, tail_runs=1, w_per=4, checks=False, scopes=False, name="gqa"):
    table, done, (n_kv, n_dkv, n_w, n_dw) = _make_plan(phases, dw_steps, defer)
    fields = list(table[0])
    n_words = (len(fields) + 3) // 4

    drips, bulk = {}, []
    for half, count in ((1, 30), (0, 54)):
        total = count * drip[0] // 4 * drip[1]
        rows = (max(total - PW, 0), min(total, PW))
        drips[half] = [(half, w) + bb + rr for w in (1, 0) for rr in _runs(drip[1], rows[w]) for bb in _runs(drip[0], 4)]
        bulk += [(half, w, 0, 4) + rr for w in (0, 1) for rr in _runs(bulk_rows, PW, rows[w])]
    assert max(defer) <= len(bulk)
    tail = _runs(out_rows, PW)[-tail_runs][0]
    stores = [(half, w, 0, 4) + rr for part in (_runs(out_rows, tail), _runs(out_rows, PW, tail))
              for half in (0, 1) for w in (0, 1) for rr in part]
    grads = [(1, rr) for rr in _runs(32, PW)]
    for j in range(DB):
        grads.insert(5 * j + 2, (0, j))

    S_KV, S_DKV, S_W, S_DW = 0, 2 * NS, 4 * NS, 5 * NS
    S_TOK = S_DW + 2 * ((NP - 1) // DB)
    S_END = S_TOK + 4

    def kernel(x_hbm, k_hbm, v_hbm, wq_hbm, wo_hbm, g_hbm,
               out_hbm, dx_hbm, dk_hbm, dv_hbm, dwq_hbm, dwo_hbm,
               x_v, g_v, kv0_v, kv1_v, dkv_v, wq_v, wo_v, dwq_v, dwo_v,
               out_acc, dx_acc, dwq_acc, dwo_acc, out_v, dx_v, qd_v, plan_s, done_s, sem):
        kv_v = (kv0_v, kv1_v)

        def cols(p):
            return pl.ds(pl.multiple_of(p * PW, 128), PW)

        def kv_copy(blk, slot, piece, s=None):
            half, w, b, nb, r, nr = piece
            s = S_KV + 2 * (blk & (NS - 1)) + half if s is None else s
            return pltpu.make_async_copy(
                (k_hbm, v_hbm)[w].at[pl.ds((blk & 1) * 4 + 8 * half + b, nb), blk >> 1, pl.ds(r, nr)],
                kv_v[half].at[pl.ds(8 * slot + 4 * w + b, nb), pl.ds(r, nr)], sem.at[s])

        def dkv_copy(blk, slot, piece):
            half, w, b, nb, r, nr = piece
            return pltpu.make_async_copy(
                dkv_v.at[slot, half, w, pl.ds(b, nb), pl.ds(r, nr)],
                (dk_hbm, dv_hbm)[w].at[pl.ds((blk & 1) * 4 + 8 * half + b, nb), blk >> 1, pl.ds(r, nr)],
                sem.at[S_DKV + 2 * (blk & (NS - 1)) + int(r >= tail)])

        def w_copy(n, w, slot):
            src = wq_hbm.at[:, cols(n >> 1)] if w == 0 else wo_hbm.at[n >> 1]
            return pltpu.make_async_copy(src, (wq_v, wo_v)[w].at[slot], sem.at[S_W + (n & (NS - 1))])

        def dw_copy(n, slot, piece):
            w, at = piece
            if w == 0:
                src, dst = dwq_v.at[slot + at], dwq_hbm.at[:, cols(DB * n + at)]
            else:
                src, dst = dwo_v.at[pl.ds(slot, DB), pl.ds(*at)], dwo_hbm.at[pl.ds(DB * n, DB), pl.ds(*at)]
            return pltpu.make_async_copy(src, dst, sem.at[S_DW + 2 * n + w])

        def tok_copies(half, c):
            return [pltpu.make_async_copy(src.at[half, c], dst.at[half, c], sem.at[S_TOK + 2 * half + w])
                    for w, (src, dst) in enumerate(((x_hbm, x_v), (g_hbm, g_v)))]

        def first_copies(b):
            return [kv_copy(0, 0, (half, w, b, 2, 0, PW), S_KV + half if b else S_END + 2 * half + w)
                    for half in (0, 1) for w in (0, 1)]

        def wait_all(buf, s):
            pltpu.make_async_copy(buf, buf, sem.at[s]).wait()

        def kv_wait(blk, _):
            for half in (0, 1):
                wait_all(kv_v[half].at[pl.ds(8 * lax.rem(blk, n_kv), 8)], S_KV + 2 * (blk & (NS - 1)) + half)

        def dkv_wait(n, _):
            slot, s = lax.rem(n >> 1, n_dkv), S_DKV + (n & (2 * NS - 1))
            pl.when((n & 1) == 0)(lambda: wait_all(dkv_v.at[slot, :, :, :, pl.ds(0, tail)], s))
            pl.when((n & 1) == 1)(lambda: wait_all(dkv_v.at[slot, :, :, :, pl.ds(tail, PW - tail)], s))

        def w_wait(n, _):
            for w in (0, 1):
                pl.when((n & 1) == w)(lambda: w_copy(n, w, lax.rem(n >> 1, n_w)).wait())

        def dw_wait(n, _):
            for w, buf in enumerate((dwq_v, dwo_v)):
                wait_all(buf.at[pl.ds(lax.rem(DB * n, n_dw), DB)], S_DW + 2 * n + w)

        def scope():
            return jax.named_scope("wait") if scopes else contextlib.nullcontext()

        def wait_until(t):
            old, new = done_s[t], done_s[t + 1]
            for n, wait in ((2, w_wait), (0, kv_wait), (3, dw_wait), (1, dkv_wait)):
                lax.fori_loop((old >> (8 * n)) & 255, (new >> (8 * n)) & 255, wait, None)

        def project(w, half, c, slot):
            return _dot(x_v[half, c], wq_v[slot]) if w == 0 else _dot(g_v[half, c], wo_v[slot], NT)

        def step(t, steps, w_slot, ahead):
            c = t & 3
            b0 = 2 * (t & 1 if len(steps) == HEAD else steps[0] % 2)
            low = lax.broadcasted_iota(jnp.int32, (SQ, 128), 1) < DH % 128
            plan = {name: (plan_s[n // 4 * NSTEP + t] >> (8 * (n % 4))) & 255 for n, name in enumerate(fields)}

            def when(name, test):
                hits = [test(table[s][name] if name else s) for s in steps]
                if all(hits) or not any(hits):
                    return lambda body: body() if hits[0] else None
                return pl.when(test(plan[name] if name else t))

            todo_drip, todo_bulk, todo_store = list(drips[1]), list(enumerate(bulk)), list(stores)
            todo_grad, todo_end = list(grads), []

            def start_some():
                for _ in range(min(2, len(todo_bulk))):
                    n, piece = todo_bulk.pop(0)
                    when("r_skip", lambda v: v <= n)(
                        lambda: kv_copy(plan["r_blk"], plan["r_slot"], piece).start(priority=1))
                for _ in range(min(w_per, len(todo_store))):
                    piece = todo_store.pop(0)
                    when("w_blk", lambda v: v != OFF)(
                        lambda: dkv_copy(plan["w_blk"], plan["w_slot"], piece).start(priority=1))
                for _ in range(min(2, len(todo_grad))):
                    piece = todo_grad.pop(0)
                    when("d_num", lambda v: v != OFF)(
                        lambda: dw_copy(plan["d_num"], plan["d_slot"], piece).start(priority=1))

            def start_end(count):
                for first, src, dst, i, j, s in todo_end[:count]:
                    when(None, lambda v: v >= first)(
                        lambda: pltpu.make_async_copy(src.at[i], dst.at[j], sem.at[S_END + s]).start())
                del todo_end[:count]

            def tick(value, r, c0=0):
                piece = todo_drip.pop(0)
                kv_v[piece[0]][8 * n_kv, 0:16, 0:128] = value[r:r + 16, c0:c0 + 128].astype(BF16)
                when("r_skip", lambda v: v != OFF)(lambda: kv_copy(plan["r_blk"], plan["r_slot"], piece).start())
                start_some()
                start_end(1 + (len(todo_end) > 4))

            def project_in(w, half, c, slot):
                r = project(w, half, c, slot)
                for n in range(3):
                    tick(r, 32 * n, 128 * n)
                return r

            def kv(w, j, tile):
                return kv_v[j // 2][8 * plan["kv_slot"] + b0 + (4 * w + j % 2), 128 * tile:128 * (tile + 1), :]

            def scores(a, w, j):
                mid = a[:, 128:256]
                mid = jnp.concatenate([jnp.where(low, mid, 0.0), jnp.where(low, 0.0, mid)], axis=0)
                m = _dot(mid.astype(BF16), kv(w, j, 1))
                s = jnp.concatenate([_dot(a[:, :128].astype(BF16), kv(w, j, 0)) + m[:SQ],
                                     _dot(a[:, 256:].astype(BF16), kv(w, j, 2)) + m[SQ:]], axis=0)
                tick(m, 0)
                tick(s, 0)
                return s

            def softmax(q, do, j):
                s = scores(q, 0, j)
                e = jnp.exp2((s - jnp.max(s, axis=1, keepdims=True)) * (DH ** -0.5 * math.log2(math.e)))
                p = e * (1.0 / jnp.sum(e, axis=1, keepdims=True))
                dp = scores(do, 1, j)
                return p, (dp - jnp.sum(p * dp, axis=1, keepdims=True)) * (p * DH ** -0.5)

            def mix(p, a, w, j):
                at = a.T.astype(BF16)
                dst = (plan["dkv_slot"], j // 2, w, b0 + j % 2)
                left = _dot(p[:SQ].astype(BF16), kv(w, j, 0), NT)
                r = _dot(at[:DH], p[:SQ].astype(BF16))
                dkv_v[dst + (pl.ds(0, DH),)] = r.astype(BF16)
                tick(left, 0)
                tick(r, 64)
                m = _dot(p.astype(BF16), kv(w, j, 1), NT)
                right = _dot(p[SQ:].astype(BF16), kv(w, j, 2), NT)
                r = _dot(at[DH:], p[SQ:].astype(BF16))
                dkv_v[dst + (pl.ds(DH, DH),)] = r.astype(BF16)
                tick(m, 0)
                tick(r, 0)
                return jnp.concatenate([left, jnp.where(low, m[:SQ], m[SQ:]), right], axis=1).astype(BF16)

            def attend(half, q, do, probs):
                o, dq = [], []
                for u, (p, ds) in enumerate(probs):
                    o.append(mix(p, do[u * SQ:(u + 1) * SQ], 1, 2 * half + u))
                    dq.append(mix(ds, q[u * SQ:(u + 1) * SQ], 0, 2 * half + u))
                for rr in _runs(out_rows, PW):
                    for w, test in enumerate((lambda v: v >> 1 == NBLK - 1, lambda v: v >= NSTEP - 2)):
                        when(None, test)(lambda: dkv_copy(
                            t >> 1, plan["dkv_slot"], (half, w, b0, 2) + rr).start(priority=1))
                return jnp.concatenate(o, axis=0), jnp.concatenate(dq, axis=0)

            def project_out(w, half, a):
                acc, res, dst = ((out_acc, out_v, out_hbm), (dx_acc, dx_v, dx_hbm))[w]
                r = _dot(a, wo_v[w_slot]) if w == 0 else _dot(a, wq_v[w_slot], NT)
                if steps[0] == 0:
                    acc[half, c] = r
                else:
                    total = acc[half, c] + r
                    acc[half, c] = total
                    res[half, c] = total.astype(BF16)
                for r0, c0 in ((0, 0), (32, 256), (112, 384)):
                    tick(r, r0, c0)
                for rr in _runs(32, 2 * SQ):
                    todo_end.append((NSTEP - 4, res, dst, (half, c, pl.ds(*rr)), (half, c, pl.ds(*rr)), w))

            def weight_grad(w, a):
                acc, res = ((dwq_acc, dwq_v), (dwo_acc, dwo_v))[w]
                tok = jnp.concatenate([(x_v, g_v)[w][half, c] for half in (0, 1)], axis=0)
                r = _dot(tok, a, TN) if w == 0 else _dot(a, tok, TN)
                total = (jnp.where(c == 0, 0.0, acc[...]) if steps[0] % 2 == 0 else acc[...]) + r
                acc[...] = total
                if steps[-1] % 2:
                    res[plan["dw_slot"]] = total.astype(BF16)
                for r0, c0 in (((0, 0), (160, 0), (320, 0), (480, 0), (0, 256), (320, 256)),
                               ((0, 0), (160, 0), (320, 0), (96, 256), (256, 256), (64, 512)))[w]:
                    tick(r, r0, c0)
                for rr in _runs(48, PW) if w else _runs(128, D):
                    j = (NP - 1, pl.ds(*rr)) if w else (pl.ds(*rr), pl.ds((NP - 1) * PW, PW))
                    todo_end.append((NSTEP - 1, res, (dwq_hbm, dwo_hbm)[w], (plan["dw_slot"], pl.ds(*rr)), j, 2 + w))

            for n in range(max(defer)):
                when("l_num", lambda v: v > n)(
                    lambda: kv_copy(plan["r_blk"] - 1, plan["l_slot"], bulk[n]).start(priority=1))
            start_some()
            q0, do0 = ahead
            q1, do1 = project_in(0, 1, c, w_slot), project_in(1, 1, c, w_slot)
            probs = [softmax(q0[u * SQ:(u + 1) * SQ], do0[u * SQ:(u + 1) * SQ], u) for u in (0, 1)]
            assert not (todo_bulk or todo_store or todo_grad)
            for half in (0, 1):
                @when(None, lambda v: v + 2 - half < 4)
                def _():
                    for copy in tok_copies(half, t + 2 - half):
                        copy.start()
            for w in (0, 1):
                when("m_mat", lambda v: (v & 0x81) == w)(
                    lambda: w_copy(plan["m_mat"], w, plan["m_slot"]).start(priority=1))
            o0, dq0 = attend(0, q0, do0, probs)

            assert not todo_drip
            todo_drip += drips[0]
            project_out(0, 0, o0)
            probs = [softmax(q1[:SQ], do1[:SQ], 2)]
            project_out(1, 0, dq0)
            probs.append(softmax(q1[SQ:], do1[SQ:], 3))
            o1, dq1 = attend(1, q1, do1, probs)
            project_out(0, 1, o1)
            weight_grad(1, jnp.concatenate([o0, o1], axis=0))
            project_out(1, 1, dq1)
            weight_grad(0, jnp.concatenate([dq0, dq1], axis=0))
            ahead = [project_in(w, 0, (c + 1) & 3, plan["w_next"]) for w in (0, 1)]
            assert not todo_drip
            start_end(len(todo_end))
            return plan["w_next"], ahead

        def one_step(t, w_slot):
            w_slot, (qd_v[0], qd_v[1]) = step(t, range(HEAD), w_slot, (qd_v[0], qd_v[1]))
            with scope():
                for half in (0, 1):
                    @pl.when(t + 2 - half < 4)
                    def _():
                        for copy in tok_copies(half, t + 2 - half):
                            copy.wait()

                @pl.when(t == 0)
                def _():
                    for copy in first_copies(2):
                        copy.wait()
                wait_until(t)
            return w_slot

        def two_steps(i, w_slot):
            w_slot, ahead = step(2 * i, range(HEAD, NSTEP, 2), w_slot, (qd_v[0], qd_v[1]))
            w_slot, (qd_v[0], qd_v[1]) = step(2 * i + 1, range(HEAD + 1, NSTEP, 2), w_slot, ahead)
            with scope():
                wait_until(2 * i + 1)
            return w_slot

        zero = jnp.int32(0)
        weights = [w_copy(zero + w, w, 0) for w in (0, 1)]
        for copy in tok_copies(0, 0) + weights + tok_copies(1, 0) + first_copies(0):
            copy.start()
        for copy in first_copies(2):
            copy.start(priority=1)
        for t, entry in enumerate(table):
            for n in range(n_words):
                plan_s[n * NSTEP + t] = _pack([entry[name] for name in fields[4 * n:4 * n + 4]])
        for t, counts in enumerate(done):
            done_s[t] = _pack(counts)
        with scope():
            for copy in tok_copies(0, 0):
                copy.wait()
            for copy in tok_copies(0, 1):
                copy.start()
            for copy in weights:
                copy.wait()
            for w in (0, 1):
                qd_v[w] = project(w, 0, 0, 0)
            for copy in tok_copies(1, 0) + tok_copies(0, 1) + first_copies(0):
                copy.wait()

        w_slot = lax.fori_loop(0, HEAD, one_step, zero)
        lax.fori_loop(HEAD // 2, NSTEP // 2, two_steps, w_slot)

        for n in range(done[-1][3], (NP - 1) // DB):
            dw_wait(zero + n, None)
        for s, buf in enumerate((out_v, dx_v, dwq_v.at[(NP - 1) % n_dw], dwo_v.at[(NP - 1) % n_dw])):
            wait_all(buf, S_END + s)
        for n in range(done[-1][1], 2 * NBLK):
            dkv_wait(zero + n, None)

    def call(x, k_cache, v_cache, wq, wo, grad_out):
        tok = (2, 4, 2 * SQ, D)
        pairs = (B, NP, PW, SK)
        hbm = pl.BlockSpec(memory_space=pl.ANY)
        out, dx, dk, dv, dwq, dwo = pl.pallas_call(
            kernel,
            out_shape=[jax.ShapeDtypeStruct(s, BF16) for s in (tok, tok, pairs, pairs, (D, NP * PW), (NP, PW, D))],
            in_specs=[hbm] * 6,
            out_specs=[hbm] * 6,
            scratch_shapes=[
                pltpu.VMEM(tok, BF16), pltpu.VMEM(tok, BF16),
                pltpu.VMEM((8 * n_kv + 1, PW, SK), BF16), pltpu.VMEM((8 * n_kv + 1, PW, SK), BF16),
                pltpu.VMEM((n_dkv, 2, 2, 4, PW, SK), BF16),
                pltpu.VMEM((n_w, D, PW), BF16), pltpu.VMEM((n_w, PW, D), BF16),
                pltpu.VMEM((n_dw, D, PW), BF16), pltpu.VMEM((n_dw, PW, D), BF16),
                pltpu.VMEM(tok, F32), pltpu.VMEM(tok, F32),
                pltpu.VMEM((D, PW), F32), pltpu.VMEM((PW, D), F32),
                pltpu.VMEM(tok, BF16), pltpu.VMEM(tok, BF16),
                pltpu.VMEM((2, 2 * SQ, PW), F32),
                pltpu.SMEM((n_words * NSTEP,), jnp.int32), pltpu.SMEM((NSTEP + 1,), jnp.int32),
                pltpu.SemaphoreType.DMA((S_END + 4,)),
            ],
            compiler_params=pltpu.CompilerParams(
                vmem_limit_bytes=128 * 1024 * 1024,
                disable_bounds_checks=checks is not True, disable_semaphore_checks=not checks),
            name=name,
        )(x.reshape(tok), jnp.swapaxes(k_cache, 2, 3).reshape(pairs), jnp.swapaxes(v_cache, 2, 3).reshape(pairs),
          wq, wo.reshape(NP, PW, D), grad_out.reshape(tok))
        dk, dv = (jnp.swapaxes(a.reshape(B, H, DH, SK), 2, 3) for a in (dk, dv))
        return out.reshape(B, SQ, D), dx.reshape(B, SQ, D), dk, dv, dwq, dwo.reshape(H * DH, D)

    return call


@jax.jit
def pallas_standalone__gqa_block_cached__near_ridge_kernel(x, k_cache, v_cache, wq, wo, grad_out):
    return make()(x, k_cache, v_cache, wq, wo, grad_out)
```

```python
import math

import jax
import jax.numpy as jnp
from jax import lax
import jax.experimental.pallas as pl
import jax.experimental.pallas.tpu as pltpu

B, SQ, D = 16, 64, 640
H, SK, DH = 32, 512, 192
NP = H // 2
PW = 2 * DH
NSTEP = 4 * NP
NBLK = NSTEP // 2
HEAD = 4
DB = 3
NS = 4
OFF = 255

PHASES = (12, 10, 10, 10, 9, 13)
DW_STEPS = (12, 32, 51, 60, 61)
DEFER = (8, 4)
TAIL = 360

NN = (((1,), (0,)), ((), ()))
NT = (((1,), (1,)), ((), ()))
TN = (((0,), (0,)), ((), ()))
F32, BF16 = jnp.float32, jnp.bfloat16


def _dot(a, b, dims=NN):
    return lax.dot_general(a, b, dims, preferred_element_type=F32)


def _runs(size, stop, start=0):
    return [(a, min(size, stop - a)) for a in range(start, stop, size)]


def _pack(fields):
    word = sum(v << (8 * n) for n, v in enumerate(fields))
    return word - (1 << 32) if word >= 1 << 31 else word


def _make_plan():
    reading = [n % 2 == 0 for n, length in enumerate(PHASES) for _ in range(length)]
    assert len(reading) == NSTEP
    switches = [t for t in range(NSTEP - 1) if reading[t] != reading[t + 1]]

    started = [(1, 0, 2, 0)]
    for t in range(NSTEP):
        r, w, m, d = started[-1]
        if reading[t]:
            r, m = r + 1, min(m + 1, 2 * NP)
        elif 2 * w + 2 <= t:
            w += 1
        if t in DW_STEPS:
            d += 1
            assert not reading[t] and DB * d <= t // 4
        started.append((r, w, m, d))
    assert started[-1] == (NBLK, NBLK - 1, 2 * NP, (NP - 1) // DB) and (NP - 1) % DB == 0

    stops = [t for t in range(NSTEP) if t < HEAD or t % 2]
    done = [(1, 0, 2, 0)]
    for t in range(NSTEP):
        r, w, m, d = done[-1]
        if t in stops[:-1]:
            until = stops[stops.index(t) + 1]
            r = max(r, until // 2 + 1, started[t + 1][0] - 2)
            m = max(m, min(2 * ((until + 1) // 4 + 1), 2 * NP), started[t + 1][2] - 2)
            w = max(w, 2 * started[t][1])
            if reading[t + 1] and not reading[t]:
                w = max(w, 2 * started[t + 1][1] - 1)
            d = max(d, started[max(t - 1, 0)][3])
        done.append((r, w, m, d))
        sr, sw, sm, sd = started[t + 1]
        assert r <= sr and w <= 2 * sw and m <= sm and d <= sd
        assert max(sr - done[t][0], sw + (t >= NSTEP - 2) - done[t][1] // 2, sm - done[t][2]) <= NS
        assert sd - done[t][3] <= 2
    for n in range(len(DEFER)):
        assert done[switches[2 * n + 1] + 1][0] < started[switches[2 * n] + 1][0]

    n_kv = max(started[t + 1][0] - t // 2 for t in range(NSTEP))
    n_dkv = max(t // 2 + 1 - done[t][1] // 2 for t in range(NSTEP))
    n_w = max((started[t + 1][2] + 1) // 2 - t // 4 for t in range(NSTEP))
    n_dw = DB * max(t // 4 // DB + 1 - done[t][3] for t in range(NSTEP))

    table = []
    for t in range(NSTEP):
        (r, w, m, d), (r1, w1, m1, d1) = started[t], started[t + 1]
        skip = sum(k for n, k in enumerate(DEFER) if t == switches[2 * n])
        late = sum(k for n, k in enumerate(DEFER) if t == switches[2 * n + 1] + 1)
        table.append(dict(
            r_blk=r, r_slot=r % n_kv, r_skip=skip if r1 > r else OFF, w_blk=w if w1 > w else OFF,
            w_slot=w % n_dkv, l_num=late, l_slot=(r - 1) % n_kv, kv_slot=t // 2 % n_kv,
            dkv_slot=t // 2 % n_dkv, dw_slot=t // 4 % n_dw, w_next=min(t + 1, NSTEP - 1) // 4 % n_w,
            m_mat=m if m1 > m else OFF, m_slot=m // 2 % n_w, d_num=d if d1 > d else OFF, d_slot=DB * d % n_dw))
    return table, done, (n_kv, n_dkv, n_w, n_dw)


def _read_pieces(drip_rows):
    drips, bulk = {}, []
    for half, count in ((1, 30), (0, 54)):
        total = count // 2 * drip_rows
        rows = (max(total - PW, 0), min(total, PW))
        drips[half] = [(half, w, b, 2) + rr for w in (1, 0) for rr in _runs(drip_rows, rows[w]) for b in (0, 2)]
        bulk += [(half, w, 0, 4) + rr for w in (0, 1) for rr in _runs(72, PW, rows[w])]
    return drips, bulk


TABLE, DONE, (N_KV, N_DKV, N_W, N_DW) = _make_plan()
FIELDS = list(TABLE[0])
N_WORDS = (len(FIELDS) + 3) // 4
OUT_RUNS = (_runs(40, TAIL), _runs(40, PW, TAIL))
STORES = [(half, w, 0, 4) + rr for part in OUT_RUNS for half in (0, 1) for w in (0, 1) for rr in part]
GRADS = [(0, n // 5) if n % 5 == 2 else (1, _runs(32, PW)[n - (n + 2) // 5]) for n in range(5 * DB)]

S_KV, S_DKV, S_W, S_DW = 0, 2 * NS, 6 * NS, 7 * NS
S_TOK = S_DW + 4
S_END = S_TOK + 4


def _kernel(x_hbm, k_hbm, v_hbm, wq_hbm, wo_hbm, g_hbm,
            out_hbm, dx_hbm, dk_hbm, dv_hbm, dwq_hbm, dwo_hbm,
            x_v, g_v, kv0_v, kv1_v, dkv_v, wq_v, wo_v, dwq_v, dwo_v,
            out_acc, dx_acc, dwq_acc, dwo_acc, out_v, dx_v, qd_v, plan_s, done_s, sem):
    kv_v = (kv0_v, kv1_v)

    def cols(p):
        return pl.ds(pl.multiple_of(p * PW, 128), PW)

    def kv_copy(blk, slot, piece, s=None):
        half, w, b, nb, r, nr = piece
        s = S_KV + 2 * (blk & (NS - 1)) + half if s is None else s
        return pltpu.make_async_copy(
            (k_hbm, v_hbm)[w].at[half, pl.ds((blk & 1) * 4 + b, nb), blk >> 1, pl.ds(r, nr)],
            kv_v[half].at[pl.ds(8 * slot + 4 * w + b, nb), pl.ds(r, nr)], sem.at[s])

    def dkv_copy(blk, slot, piece):
        half, w, b, nb, r, nr = piece
        return pltpu.make_async_copy(
            dkv_v.at[slot, w, half, pl.ds(b, nb), pl.ds(r, nr)],
            (dk_hbm, dv_hbm)[w].at[half, pl.ds((blk & 1) * 4 + b, nb), blk >> 1, pl.ds(r, nr)],
            sem.at[S_DKV + 4 * (blk & (NS - 1)) + 2 * int(r >= TAIL) + w])

    def w_copy(n, w, slot):
        src = wq_hbm.at[:, cols(n >> 1)] if w == 0 else wo_hbm.at[n >> 1]
        return pltpu.make_async_copy(src, (wq_v, wo_v)[w].at[slot], sem.at[S_W + (n & (NS - 1))])

    def dw_copy(n, slot, piece):
        w, at = piece
        if w == 0:
            src, dst = dwq_v.at[slot + at], dwq_hbm.at[:, cols(DB * n + at)]
        else:
            src, dst = dwo_v.at[pl.ds(slot, DB), pl.ds(*at)], dwo_hbm.at[pl.ds(DB * n, DB), pl.ds(*at)]
        return pltpu.make_async_copy(src, dst, sem.at[S_DW + 2 * (n & 1) + w])

    def last_copy(w, at):
        if w < 2:
            src, dst = (out_v, dx_v)[w].at[at], (out_hbm, dx_hbm)[w].at[at]
        elif w == 2:
            src, dst = dwq_v.at[(NP - 1) % N_DW, at], dwq_hbm.at[at, pl.ds((NP - 1) * PW, PW)]
        else:
            src, dst = dwo_v.at[(NP - 1) % N_DW, at], dwo_hbm.at[NP - 1, at]
        return pltpu.make_async_copy(src, dst, sem.at[S_END + w])

    def tok_copies(half, c):
        return [pltpu.make_async_copy(src.at[half, c], dst.at[half, c], sem.at[S_TOK + 2 * half + w])
                for w, (src, dst) in enumerate(((x_hbm, x_v), (g_hbm, g_v)))]

    def first_copies(b):
        return [kv_copy(0, 0, (half, w, b, 2, 0, PW), (S_DW if b else S_END) + 2 * half + w)
                for half in (0, 1) for w in (0, 1)]

    def kv_wait(blk, _):
        for half in (0, 1):
            buf = kv_v[half].at[pl.ds(8 * lax.rem(blk, N_KV), 8)]
            pltpu.make_async_copy(buf, buf, sem.at[S_KV + 2 * (blk & (NS - 1)) + half]).wait()

    def dkv_wait(n, _):
        for part, rows in enumerate(((0, TAIL), (TAIL, PW - TAIL))):
            @pl.when((n & 1) == part)
            def _():
                for w in (0, 1):
                    dkv_copy(n >> 1, lax.rem(n >> 1, N_DKV), (pl.ds(0, 2), w, 0, 4) + rows).wait()

    def w_wait(n, _):
        for w in (0, 1):
            pl.when((n & 1) == w)(lambda: w_copy(n, w, lax.rem(n >> 1, N_W)).wait())

    def dw_wait(n, _):
        for piece in [(0, j) for j in range(DB)] + [(1, (0, PW))]:
            dw_copy(n, lax.rem(DB * n, N_DW), piece).wait()

    def wait_until(t):
        old, new = done_s[t], done_s[t + 1]
        for n, wait in ((2, w_wait), (0, kv_wait), (3, dw_wait), (1, dkv_wait)):
            lax.fori_loop((old >> (8 * n)) & 255, (new >> (8 * n)) & 255, wait, None)

    def project(w, half, c, slot):
        return _dot(x_v[half, c], wq_v[slot]) if w == 0 else _dot(g_v[half, c], wo_v[slot], NT)

    def step(t, steps, w_slot, ahead):
        head = steps[0] == 0
        c = t & 3
        b0 = 2 * (t & 1 if head else steps[0] % 2)
        low = lax.broadcasted_iota(jnp.int32, (SQ, 128), 1) < DH % 128
        plan = {name: (plan_s[n // 4 * NSTEP + t] >> (8 * (n % 4))) & 255 for n, name in enumerate(FIELDS)}

        def when(name, test):
            hits = [test(TABLE[s][name] if name else s) for s in steps]
            if all(hits) or not any(hits):
                return lambda body: body() if hits[0] else None
            return pl.when(test(plan[name] if name else t))

        drips, bulk = _read_pieces(16 if head else 24)
        todo_drip, todo_bulk, todo_store = list(drips[1]), list(enumerate(bulk)), list(STORES)
        todo_grad, todo_last = list(GRADS), []

        def start_some():
            for _ in range(min(2, len(todo_bulk))):
                n, piece = todo_bulk.pop(0)
                when("r_skip", lambda v: v <= n)(
                    lambda: kv_copy(plan["r_blk"], plan["r_slot"], piece).start(priority=1))
            for _ in range(min(4, len(todo_store))):
                piece = todo_store.pop(0)
                when("w_blk", lambda v: v != OFF)(
                    lambda: dkv_copy(plan["w_blk"], plan["w_slot"], piece).start(priority=1))
            for _ in range(min(2, len(todo_grad))):
                piece = todo_grad.pop(0)
                when("d_num", lambda v: v != OFF)(
                    lambda: dw_copy(plan["d_num"], plan["d_slot"], piece).start(priority=1))

        def start_last(count):
            for first, w, at in todo_last[:count]:
                when(None, lambda v: v >= first)(lambda: last_copy(w, at).start())
            del todo_last[:count]

        def tick(value, r, c0=0):
            piece = todo_drip.pop(0)
            kv_v[piece[0]][8 * N_KV, 0:16, 0:128] = value[r:r + 16, c0:c0 + 128].astype(BF16)
            when("r_skip", lambda v: v != OFF)(lambda: kv_copy(plan["r_blk"], plan["r_slot"], piece).start())
            start_some()
            start_last(1 + (len(todo_last) > 4))

        def project_in(w, half, c, slot):
            r = project(w, half, c, slot)
            for n in range(3):
                tick(r, 32 * n, 128 * n)
            return r

        def kv(w, j, tile):
            return kv_v[j // 2][8 * plan["kv_slot"] + b0 + (4 * w + j % 2), 128 * tile:128 * (tile + 1), :]

        def scores(a, w, j):
            mid = a[:, 128:256]
            mid = jnp.concatenate([jnp.where(low, mid, 0.0), jnp.where(low, 0.0, mid)], axis=0)
            m = _dot(mid.astype(BF16), kv(w, j, 1))
            s = jnp.concatenate([_dot(a[:, :128].astype(BF16), kv(w, j, 0)) + m[:SQ],
                                 _dot(a[:, 256:].astype(BF16), kv(w, j, 2)) + m[SQ:]], axis=0)
            tick(m, 0)
            tick(s, 0)
            return s

        def softmax(q, do, j):
            s = scores(q, 0, j)
            e = jnp.exp2((s - jnp.max(s, axis=1, keepdims=True)) * (DH ** -0.5 * math.log2(math.e)))
            p = e * (1.0 / jnp.sum(e, axis=1, keepdims=True))
            dp = scores(do, 1, j)
            return p, (dp - jnp.sum(p * dp, axis=1, keepdims=True)) * (p * DH ** -0.5)

        def mix(p, a, w, j):
            at = a.T.astype(BF16)
            dst = (plan["dkv_slot"], w, j // 2, b0 + j % 2)
            left = _dot(p[:SQ].astype(BF16), kv(w, j, 0), NT)
            r = _dot(at[:DH], p[:SQ].astype(BF16))
            dkv_v[dst + (pl.ds(0, DH),)] = r.astype(BF16)
            tick(left, 0)
            tick(r, 64)
            m = _dot(p.astype(BF16), kv(w, j, 1), NT)
            right = _dot(p[SQ:].astype(BF16), kv(w, j, 2), NT)
            r = _dot(at[DH:], p[SQ:].astype(BF16))
            dkv_v[dst + (pl.ds(DH, DH),)] = r.astype(BF16)
            tick(m, 0)
            tick(r, 0)
            return jnp.concatenate([left, jnp.where(low, m[:SQ], m[SQ:]), right], axis=1).astype(BF16)

        def attend(half, q, do, probs):
            o, dq = [], []
            for u, (p, ds) in enumerate(probs):
                o.append(mix(p, do[u * SQ:(u + 1) * SQ], 1, 2 * half + u))
                dq.append(mix(ds, q[u * SQ:(u + 1) * SQ], 0, 2 * half + u))
            for rr in OUT_RUNS[0] + OUT_RUNS[1]:
                for w, test in enumerate((lambda v: v >> 1 == NBLK - 1, lambda v: v >= NSTEP - 2)):
                    when(None, test)(lambda: dkv_copy(
                        t >> 1, plan["dkv_slot"], (half, w, b0, 2) + rr).start(priority=1))
            return jnp.concatenate(o, axis=0), jnp.concatenate(dq, axis=0)

        def project_out(w, half, a):
            acc, res = ((out_acc, out_v), (dx_acc, dx_v))[w]
            r = _dot(a, wo_v[w_slot]) if w == 0 else _dot(a, wq_v[w_slot], NT)
            if head:
                acc[half, c] = r
            else:
                total = acc[half, c] + r
                acc[half, c] = total
                res[half, c] = total.astype(BF16)
            for r0, c0 in ((0, 0), (32, 256), (112, 384)):
                tick(r, r0, c0)
            todo_last.extend((NSTEP - 4, w, (half, c, pl.ds(*rr))) for rr in _runs(32, 2 * SQ))

        def weight_grad(w, a):
            acc, res = ((dwq_acc, dwq_v), (dwo_acc, dwo_v))[w]
            tok = jnp.concatenate([(x_v, g_v)[w][half, c] for half in (0, 1)], axis=0)
            r = _dot(tok, a, TN) if w == 0 else _dot(a, tok, TN)
            total = (jnp.where(c == 0, 0.0, acc[...]) if steps[0] % 2 == 0 else acc[...]) + r
            acc[...] = total
            if steps[-1] % 2:
                res[plan["dw_slot"]] = total.astype(BF16)
            for r0, c0 in (((0, 0), (160, 0), (320, 0), (480, 0), (0, 256), (320, 256)),
                           ((0, 0), (160, 0), (320, 0), (96, 256), (256, 256), (64, 512)))[w]:
                tick(r, r0, c0)
            todo_last.extend((NSTEP - 1, 2 + w, pl.ds(*rr)) for rr in (_runs(48, PW) if w else _runs(128, D)))

        for n in range(max(DEFER)):
            when("l_num", lambda v: v > n)(
                lambda: kv_copy(plan["r_blk"] - 1, plan["l_slot"], bulk[n]).start(priority=1))
        start_some()
        q0, do0 = ahead
        q1, do1 = project_in(0, 1, c, w_slot), project_in(1, 1, c, w_slot)
        probs = [softmax(q0[u * SQ:(u + 1) * SQ], do0[u * SQ:(u + 1) * SQ], u) for u in (0, 1)]
        assert not (todo_bulk or todo_store or todo_grad)
        for half in (0, 1):
            @when(None, lambda v: v + 2 - half < 4)
            def _():
                for copy in tok_copies(half, t + 2 - half):
                    copy.start()
        for w in (0, 1):
            when("m_mat", lambda v: (v & 0x81) == w)(
                lambda: w_copy(plan["m_mat"], w, plan["m_slot"]).start(priority=1))
        o0, dq0 = attend(0, q0, do0, probs)

        assert not todo_drip
        todo_drip += drips[0]
        project_out(0, 0, o0)
        probs = [softmax(q1[:SQ], do1[:SQ], 2)]
        project_out(1, 0, dq0)
        probs.append(softmax(q1[SQ:], do1[SQ:], 3))
        o1, dq1 = attend(1, q1, do1, probs)
        project_out(0, 1, o1)
        weight_grad(1, jnp.concatenate([o0, o1], axis=0))
        project_out(1, 1, dq1)
        weight_grad(0, jnp.concatenate([dq0, dq1], axis=0))
        ahead = [project_in(w, 0, (c + 1) & 3, plan["w_next"]) for w in (0, 1)]
        assert not todo_drip
        start_last(len(todo_last))
        return plan["w_next"], ahead

    def one_step(t, w_slot):
        w_slot, (qd_v[0], qd_v[1]) = step(t, range(HEAD), w_slot, (qd_v[0], qd_v[1]))
        for half in (0, 1):
            @pl.when(t + 2 - half < 4)
            def _():
                for copy in tok_copies(half, t + 2 - half):
                    copy.wait()

        @pl.when(t == 0)
        def _():
            for copy in first_copies(2):
                copy.wait()
        wait_until(t)
        return w_slot

    def two_steps(i, w_slot):
        w_slot, ahead = step(2 * i, range(HEAD, NSTEP, 2), w_slot, (qd_v[0], qd_v[1]))
        w_slot, (qd_v[0], qd_v[1]) = step(2 * i + 1, range(HEAD + 1, NSTEP, 2), w_slot, ahead)
        wait_until(2 * i + 1)
        return w_slot

    zero = jnp.int32(0)
    weights = [w_copy(zero + w, w, 0) for w in (0, 1)]
    for copy in tok_copies(0, 0) + weights + tok_copies(1, 0) + first_copies(0):
        copy.start()
    for t, entry in enumerate(TABLE):
        for n in range(N_WORDS):
            plan_s[n * NSTEP + t] = _pack([entry[name] for name in FIELDS[4 * n:4 * n + 4]])
    for t, counts in enumerate(DONE):
        done_s[t] = _pack(counts)
    for copy in tok_copies(0, 0):
        copy.wait()
    for copy in tok_copies(0, 1):
        copy.start()
    for copy in first_copies(2):
        copy.start(priority=1)
    for copy in weights:
        copy.wait()
    for w in (0, 1):
        qd_v[w] = project(w, 0, 0, 0)
    for copy in tok_copies(1, 0) + tok_copies(0, 1) + first_copies(0):
        copy.wait()

    w_slot = lax.fori_loop(0, HEAD, one_step, zero)
    lax.fori_loop(HEAD // 2, NSTEP // 2, two_steps, w_slot)

    for n in range(DONE[-1][3], (NP - 1) // DB):
        dw_wait(zero + n, None)
    for w, whole in enumerate((2, 2, D, PW)):
        last_copy(w, pl.ds(0, whole)).wait()
    for n in range(DONE[-1][1], 2 * NBLK):
        dkv_wait(zero + n, None)


@jax.jit
def pallas_standalone__gqa_block_cached__near_ridge_kernel(
    x: jax.Array,
    k_cache: jax.Array,
    v_cache: jax.Array,
    wq: jax.Array,
    wo: jax.Array,
    grad_out: jax.Array,
):
    tok = (2, 4, 2 * SQ, D)
    pairs = (2, B // 2, NP, PW, SK)
    hbm = pl.BlockSpec(memory_space=pl.ANY)
    out, dx, dk, dv, dwq, dwo = pl.pallas_call(
        _kernel,
        out_shape=[jax.ShapeDtypeStruct(s, BF16) for s in (tok, tok, pairs, pairs, (D, NP * PW), (NP, PW, D))],
        in_specs=[hbm] * 6,
        out_specs=[hbm] * 6,
        scratch_shapes=[
            pltpu.VMEM(tok, BF16), pltpu.VMEM(tok, BF16),
            pltpu.VMEM((8 * N_KV + 1, PW, SK), BF16), pltpu.VMEM((8 * N_KV + 1, PW, SK), BF16),
            pltpu.VMEM((N_DKV, 2, 2, 4, PW, SK), BF16),
            pltpu.VMEM((N_W, D, PW), BF16), pltpu.VMEM((N_W, PW, D), BF16),
            pltpu.VMEM((N_DW, D, PW), BF16), pltpu.VMEM((N_DW, PW, D), BF16),
            pltpu.VMEM(tok, F32), pltpu.VMEM(tok, F32),
            pltpu.VMEM((D, PW), F32), pltpu.VMEM((PW, D), F32),
            pltpu.VMEM(tok, BF16), pltpu.VMEM(tok, BF16),
            pltpu.VMEM((2, 2 * SQ, PW), F32),
            pltpu.SMEM((N_WORDS * NSTEP,), jnp.int32), pltpu.SMEM((NSTEP + 1,), jnp.int32),
            pltpu.SemaphoreType.DMA((S_END + 4,)),
        ],
        compiler_params=pltpu.CompilerParams(vmem_limit_bytes=128 * 1024 * 1024, disable_bounds_checks=True),
        name="gqa_block_fwd_bwd",
    )(x.reshape(tok), jnp.swapaxes(k_cache, 2, 3).reshape(pairs), jnp.swapaxes(v_cache, 2, 3).reshape(pairs),
      wq, wo.reshape(NP, PW, D), grad_out.reshape(tok))
    dk, dv = (jnp.swapaxes(a.reshape(B, H, DH, SK), 2, 3) for a in (dk, dv))
    return out.reshape(B, SQ, D), dx.reshape(B, SQ, D), dk, dv, dwq, dwo.reshape(H * DH, D)
```
